```python
import os as _os
_os.environ.setdefault("JAX_PLATFORMS", "cpu")
import jax
import jax.numpy as jnp

def _softmax(x, axis=-1):
    return jax.nn.softmax(x, axis=axis)
def _gelu(x):
    return jax.nn.gelu(x, approximate=True)
def _silu(x):
    return jax.nn.silu(x)
def _sigmoid(x):
    return jax.nn.sigmoid(x)
def _layernorm(x, axis=-1, eps=1e-5):
    m = jnp.mean(x, axis=axis, keepdims=True)
    v = jnp.var(x, axis=axis, keepdims=True)
    return (x - m) / jnp.sqrt(v + eps)
def _scatter_add(tgt, idx, src, axis=0):
    return tgt.at[idx].add(src)
def _segment_sum(src, seg, n):
    return jax.ops.segment_sum(src, seg, n)
class _Rng:
    def __init__(self, key):
        self._k = key
    def _next(self):
        self._k, sub = jax.random.split(self._k)
        return sub
    def normal(self, shape):
        return jax.random.normal(self._next(), shape, dtype=jnp.bfloat16)
    def randint(self, lo, hi, shape):
        return jax.random.randint(self._next(), shape, lo, hi, dtype=jnp.int32)
    def uniform(self, shape, lo=0.0, hi=1.0):
        return jax.random.uniform(self._next(), shape, jnp.bfloat16, lo, hi)
    def permutation(self, n):
        return jax.random.permutation(self._next(), n)


kernel_name = 'standalone__mixer_token_mlp__sampling'

def setup_inputs():
    _rng = _Rng(jax.random.key(int.from_bytes(__import__("os").urandom(4), "little")))
    _w = (lambda a: (lambda t: t.astype(jnp.bfloat16) if jnp.issubdtype(t.dtype, jnp.floating) else t)(jnp.asarray(a)))
    B, S, D, F = 32, 16, 1024, 3584
    return {
        "x": _w((lambda *s: _rng.normal(s) * 0.05)(B, S, D)),
        "w1": _w((lambda *s: _rng.normal(s) * 0.05)(S, F) * (S ** -0.5)),
        "b1": _w((lambda *s: _rng.normal(s) * 0.05)(F) * 0.02),
        "w2": _w((lambda *s: _rng.normal(s) * 0.05)(F, S) * (F ** -0.5)),
        "b2": _w((lambda *s: _rng.normal(s) * 0.05)(S) * 0.02),
    }

def reference(x, w1, b1, w2, b2):
    B, S, D = x.shape
    h = _layernorm(x, axis=-1)
    u = jnp.einsum("bsd,sf->bdf", h, w1) + b1
    u = _gelu(u)
    y = jnp.einsum("bdf,fs->bds", u, w2) + b2
    return (lambda x, *d: x.transpose(*d))(y, 0, 2, 1)
```

```python
import functools, numpy as np, ml_dtypes
import jax, jax.numpy as jnp
from jax import lax
import jax.experimental.pallas as pl
import jax.experimental.pallas.tpu as pltpu

C0 = float(np.sqrt(2/np.pi)); C1 = C0*0.044715
A = float(np.cbrt(C1)); KK = C0/A
def _bf(v): return float(np.float32(v).astype(ml_dtypes.bfloat16))
A0 = _bf(A); A1 = _bf(A-A0); A2 = _bf(A-A0-A1)
f32 = jnp.float32; bf16 = jnp.bfloat16
FC = 128; DC = 512; NJ = 4; NF = 28; NB = 8
pk = lambda a: pltpu.bitcast(a.astype(bf16), f32)
upk = lambda a: pltpu.bitcast(a, bf16)

def plan(n, vw, ss, gs, lag, hole, hpos, wy, tail, slack):
    m = 16//ss; per = (NJ//vw)*m
    flat = [4*vw*ss for _ in range(per*(n+1))]
    for q in range(m, per*n+1, m):
        if gs > 1: flat[q] += 6*vw; flat[q+gs-1] += 4*vw
        else: flat[q] += 10*vw
    total = sum(flat)
    R = [0]*NF; i = 0
    for k in range(n):
        t = sum(flat[:(k+1)*per+gs])/total*(NF+tail) + slack - 1
        i = min(max(i, int(np.ceil(t-1e-9))), NF-(n-k)); R[i] = 1; i += 1
    stream = [(c, b) for c in range(NF) for b in range(NB-1, R[c]-1, -1)]
    L = len(stream)
    last = np.cumsum([NB-r for r in R])
    cut = [int(last[c]) + lag for c in range(NF)]
    cut = [cut[-1]-L] + cut
    dots = [[(q//L,)+stream[q % L] for q in range(cut[t], cut[t+1])] for t in range(NF)]
    W = [[1 + (hole if k == hpos else 0) for k in range(len(d))] + [wy] for d in dots]
    scale = total/(sum(map(sum, W))*(1+tail/NF))
    due = np.cumsum(R)*per + gs*(np.cumsum(R) > 0)
    cnt = []; q = 0; credit = 0.0
    for t in range(NF):
        row = []
        for k, w in enumerate(W[t]):
            credit += w*scale; c = 0
            need = due[t] if k == len(W[t])-2 else (len(flat) if (t, k) == (NF-1, len(W[t])-1) else 0)
            while q < len(flat) and (credit >= flat[q]/2 or q < need): credit -= flat[q]; q += 1; c += 1
            row.append(c)
        cnt.append(row)
    return R, dots, cnt, stream[:cut[0]]

def make(n=16, BB=1, flags=None, vw=1, ss=1, gs=5, gm='mix', lag=9, hole=0, hpos=4, wy=1, tail=0.0, slack=0.5, lnpos=20, cnt=None, trips=None):
    R, dots, cnt0, head = plan(n, vw, ss, gs, lag, hole, hpos, wy, tail, slack)
    cnt = cnt or [cnt0]*(2*BB)
    vidx = np.concatenate([[0], np.cumsum(R)])
    def ln(x):
        x = x.astype(f32)
        m = jnp.mean(x, axis=-1, keepdims=True)
        xc = x - m
        v = jnp.mean(xc*xc, axis=-1, keepdims=True)
        return (xc * (lax.rsqrt(v + 1e-5)*A)).astype(bf16)
    def act(u):
        return u*jnp.tanh(u*(KK + u*u))
    def kern(x_hbm, w1_ref, b1_ref, w2t_ref, b2_ref, o_hbm, x_s, o_s, sem, w_s, b_s, hf_s, h_s, one_s, g_s):
        S, F = w1_ref.shape; B, _, D = x_s.shape
        nd = D//DC; nit = trips or B//BB
        W2O = F//2; GV = W2O + NF*8; DUM = GV + 4*NJ*16
        wb = lambda q, s: 16*(17*q + s)
        n0 = BB+1
        cp0 = pltpu.make_async_copy(x_hbm.at[0:n0], x_s.at[0:n0], sem.at[0]); cp0.start()
        cp1 = pltpu.make_async_copy(x_hbm.at[n0:B], x_s.at[n0:B], sem.at[1]); cp1.start()
        b1 = b1_ref[...].astype(f32)
        row = lax.broadcasted_iota(jnp.int32, (16, F), 0)
        w1a = jnp.concatenate([w1_ref[...].astype(f32), jnp.where(row < 3, b1, 0.0)], axis=0)
        w1t = w1a.T
        w_s[0:F//2, 0:32] = pk(w1t)
        for k in range(NF):
            w_s[W2O+8*k:W2O+8*k+8, :] = pk(w2t_ref[:, k*FC:(k+1)*FC])
        p = lax.dot_general(w2t_ref[...], w1a.astype(bf16), (((1,),(1,)),((),())), preferred_element_type=f32)
        lane = lax.broadcasted_iota(jnp.int32, (16, 16), 1); rw = lax.broadcasted_iota(jnp.int32, (16, 16), 0)
        b2c = jnp.sum(jnp.where(lane == rw, b2_ref[...].astype(f32), 0.0), axis=1, keepdims=True)
        for s in range(16):
            b_s[wb(n,s):wb(n,s)+16, :] = jnp.broadcast_to(p[:, s:s+1], (16,128))
        b_s[wb(n,16):wb(n,16)+16, :] = jnp.broadcast_to(p[:, 16:17]*A + b2c*(2*A), (16,128))
        for k in range(NF):
            if R[k]:
                blk = w1t[k*FC:k*FC+16, :]; o = int(vidx[k])
                for s in range(17):
                    c = jnp.broadcast_to(blk[:, s:s+1], (16,128))
                    b_s[wb(o,s):wb(o,s)+16, :] = c*A if s == 16 else c
        rowd = lax.broadcasted_iota(jnp.int32, (16, DC), 0)
        one_s[...] = pk(jnp.where(rowd == 0, A0, jnp.where(rowd == 1, A1, jnp.where(rowd == 2, A2, 0.0))))
        def put_h(h, dc):
            hh = h[:, dc*DC:(dc+1)*DC]
            h_s[:, dc*DC:(dc+1)*DC] = pk(hh)
            hf_s[:, dc*DC:(dc+1)*DC] = hh.astype(f32)
        def mm1(ls, dc):
            h = upk(jnp.concatenate([h_s[:, dc*DC:(dc+1)*DC], one_s[...]], axis=0))
            u = jnp.dot(upk(jnp.concatenate(ls, axis=0)), h, preferred_element_type=f32)
            return [act(u[r:r+16]) for r in range(0, u.shape[0], 16)]
        lhs = lambda c, b: w_s[(c*NB+b)*8:(c*NB+b)*8+8, 0:32]
        cp0.wait()
        h0 = ln(x_s[0]); put_h(h0, 0); put_h(h0, 1)
        for i, g in enumerate(mm1([lhs(c, b) for c, b in head], 0)): g_s[i] = g
        out0 = pltpu.make_async_copy(o_s.at[0:B-BB], o_hbm.at[0:B-BB], sem.at[2])
        out1 = pltpu.make_async_copy(o_s.at[B-BB:B], o_hbm.at[B-BB:B], sem.at[3])
        def body(it, carry):
            @pl.when(it == 1)
            def _(): cp1.wait()
            @pl.when(it == nit-1)
            def _(): out0.start()
            za = it >> 20
            na_ = [0]
            def anchor(v):
                w_s[pl.ds(pl.multiple_of(za*8 + DUM + 8*na_[0], 8), 8), :] = v; na_[0] = (na_[0]+1) % 256
            def fin(cols, jb, j0):
                zs = [u*(KK + u*u) for u in cols]
                if gs > 1:
                    yield [z[r:r+8] for z in zs for r in (0,8)]
                    for _ in range(gs-2): yield []
                for j, (u, z) in enumerate(zip(cols, zs)):
                    w_s[pl.ds(pl.multiple_of(za*8 + GV + ((jb % 4)*NJ + j0 + j)*16, 8), 16), :] = u*jnp.tanh(z)
                yield []
            def vpu(dc, res):
                defer = iter(())
                for q in range(n+1):
                    for j0 in range(0, NJ, vw):
                        accs = {}
                        for s in range(16):
                            ws = [b_s[wb(q,s)+8*a:wb(q,s)+8*a+8, :] for a in range(2)]
                            for j in range(j0, j0+vw):
                                hb = jnp.broadcast_to(hf_s[s:s+1, dc*DC+j*128:dc*DC+(j+1)*128], (8,128))
                                for a in range(2):
                                    p = accs.get((a,j))
                                    if p is None and q < n: p = b_s[wb(q,16)+8*a:wb(q,16)+8*a+8, :]
                                    accs[(a,j)] = ws[a]*hb if p is None else p + ws[a]*hb
                            if s == 15:
                                cols = [jnp.concatenate([accs[(0,j)], accs[(1,j)]], axis=0) for j in range(j0, j0+vw)]
                                if q == n: res.extend(cols)
                            if s % ss == ss-1: yield list(accs.values()), next(defer, [])
                        if q < n: defer = fin(cols, q, j0)
            G = {cb: g_s[i] for i, cb in enumerate(head)}
            for bb in range(BB):
                b = it*BB + bb
                for dc in range(nd):
                    res = []; gen = vpu(dc, res); done = []
                    def run(m):
                        for i in range(m):
                            vs, ex = next(gen); done.append(0)
                            for v in ex: anchor(v)
                            if i == m-1 or len(done) % (16//ss) == 0:
                                for v in vs: anchor(v)
                    acc = jnp.concatenate([b_s[wb(n,16):wb(n,16)+16, :]]*NJ, axis=1)
                    cn = cnt[bb*nd+dc]
                    for t in range(NF):
                        if (dc, t) == (nd-1, lnpos):
                            hn = ln(x_s[jnp.minimum(b+1, B-1)]); put_h(hn, 0)
                        k = 0
                        for nx in (0, 1):
                            part = [e for e in dots[t] if e[0] == nx]
                            if not part: continue
                            ls = []
                            for _, c, blk in part:
                                ls.append(lhs(c, blk)); run(cn[t][k]); k += 1
                            for (_, c, blk), g in zip(part, mm1(ls, (dc+nx) % nd)):
                                if nx and bb == BB-1 and dc == nd-1: g_s[head.index((c, blk))] = g
                                else: G[(c, blk)] = g
                        if R[t]:
                            o = GV + (int(vidx[t]) % 4)*NJ*16
                            G[(t, 0)] = jnp.concatenate([w_s[o+16*j:o+16*j+16, :] for j in range(NJ)], axis=1)
                        g = jnp.concatenate([G.pop((t, blk)) for blk in range(NB)], axis=0)
                        if gm == 'f32': g = g.astype(bf16)
                        acc = acc + lax.dot_general(upk(w_s[W2O+8*t:W2O+8*t+8, :]), g, (((1,),(0,)),((),())), preferred_element_type=f32)
                        run(cn[t][-1])
                    acc = acc + jnp.concatenate(res, axis=1)
                    o_s[b, :, dc*DC:(dc+1)*DC] = ((0.5/A)*acc).astype(o_s.dtype)
                put_h(hn, 1)
            return carry
        lax.fori_loop(0, nit, body, 0)
        out1.start(); out0.wait(); out1.wait()
    @jax.jit
    def fn(x, w1, b1, w2, b2):
        B,S,D = x.shape; F = w1.shape[1]
        vm = pl.BlockSpec(memory_space=pltpu.VMEM); hb = pl.BlockSpec(memory_space=pl.ANY)
        return pl.pallas_call(kern,
            in_specs=[hb, vm, vm, vm, vm], out_specs=hb,
            out_shape=jax.ShapeDtypeStruct(x.shape, x.dtype),
            scratch_shapes=[pltpu.VMEM(x.shape, x.dtype), pltpu.VMEM(x.shape, x.dtype), pltpu.SemaphoreType.DMA((4,)),
                            pltpu.VMEM((F//2+F//16+4*NJ*16+2048,128), f32), pltpu.VMEM((17*16*(n+1),128), f32), pltpu.VMEM((16,D), f32),
                            pltpu.VMEM((8,D), f32), pltpu.VMEM((8,DC), f32), pltpu.VMEM((len(head),16,DC), f32)],
            compiler_params=pltpu.CompilerParams(vmem_limit_bytes=64*2**20, flags=flags),
        )(x, w1, b1.reshape(1,F), w2.T, b2.reshape(1,S))
    return fn


_impl = make(n=19)


@jax.jit
def pallas_standalone__mixer_token_mlp__sampling_kernel(x, w1, b1, w2, b2):
    return _impl(x, w1, b1, w2, b2)
```

```python
import functools

import numpy as np
import jax
import jax.numpy as jnp
from jax import lax
import jax.experimental.pallas as pl
import jax.experimental.pallas.tpu as pltpu

F32, BF16 = jnp.float32, jnp.bfloat16

_C0 = float(np.sqrt(2.0 / np.pi))
GELU_A = float(np.cbrt(_C0 * 0.044715))
GELU_K = _C0 / GELU_A
EPS = 1e-5


def _bf16_parts(v, n):
    parts = []
    for _ in range(n):
        bits = np.array(v, np.float32).view(np.uint32) & np.uint32(0xFFFF0000)
        parts.append(float(bits.view(np.float32)))
        v -= parts[-1]
    return parts


A_PARTS = _bf16_parts(GELU_A, 3)

LANES = 128
BLK = 16
NBLK = 8
GROUP = 512
NCOL = GROUP // LANES
KAUG = 24
STEPS = 56
NPIN = 64


UNROLL = 6
NSLOT = 2
LAG = 9
GELU_DELAY = 4
RELOAD_AT = 1
PREP_AHEAD, LIN_AT, STATS_AT, STATS_PACE = 4, 5, 12, (1, 3, 8)
NORM_AT, NORM_PACE = (0, 7), 115
TILES = [int(c) for c in "0010111101110111101111011111"]
N_VPU = sum(TILES)
SLICES = {
    ("first", 1):
        "25b4a764867466650a5466456884055565a648124b767554329586484574445514957356577a8435"
        "1359556640683865549674853458a263519577762920975666447457555593415595698145464977"
        "555507685611758366546973684682b60a2421c5798670725566666446544595441b400",
    ("loop", 0):
        "34a68556a66556651a5466456944545555a6472626758664428684675372557516a5735555696645"
        "406a5466427a6565546743556558a263555577755620985666447457555592545775496443456777"
        "754447655616568365515e33684664a5554445a3565663855556667446554585444b100",
    ("loop", 1):
        "34a68556a66556651a5466456944545555a6472546856664428684675374547416a5735555696645"
        "406a5467417a6565546743556558a263555577755620985666447457555592545775396543456777"
        "754447655616568366542b73484664a5554445a55656618555566674465545854449300",
    ("loop", 2):
        "34a68556a66556651a5465456944546552d6472546856664428684675374546516a5735555695655"
        "406a5467336a6565546743556558a263555577765610985666447457555592545775396543456777"
        "754447655806568366442b73484664a5554445a5565661855556667446554585444b100",
    ("loop", 3):
        "34a68556a66754651a5466426937555555a6472546856664428684675074746526a5735555696645"
        "406a5466427a6565546743556528a293556576755620985666447457555592545775396543456777"
        "554467655616568266542b73584662a5554645a5565661855556667446554585444b100",
    ("loop", 4):
        "34a68556a66556612a8466455927545555a6472546856665428584675374546516a5474555696645"
        "406a5466427a6268546743556558a263555577755620985666447457555592545775496443456777"
        "754447655616568364542b455b3664a5554445a5565661856456667446554585444b100",
    ("loop", 5):
        "34a68556756656651d5466456944535565a6472546856664428684675374546516a5735555696645"
        "404a7466427a6565546743556558a263555577755620985666447457555592545775396543456777"
        "754447655616566366543b74484665a555444595565661855556667446554585444b100",
    ("loop", 6):
        "54a6655856935683477466446a17455346a945354595866442856567255944472596735555693647"
        "424c5266424a956545656356660ca163556577608616758565557186644392855675496443456746"
        "757448655616568357355d3348296495554435928684546635476684475545834469030",
    ("loop", 7):
        "34a68556a66754651a5466456934555555a6472546856664428684675074746426a5745555696645"
        "406a5466427a6565546743556518a293556676755620985666447457555592545775396543456777"
        "554467655616577257542b73584662a5554645a5465662857566664445524577545b110",
    ("loop", 8):
        "54a6655676935683277466446c17455346a945354595866442856567255954471596735555693647"
        "424c52664259956544666356660ca163556577707616749566457156644692855675496443456746"
        "457358955616568356575b13492864a5554453928684546635476684475545834469120",
    ("loop", 9):
        "54a6653876935683477466446a17455346a945354595686442856567155a54471596733557693647"
        "424c5266424a956544666356671c8163556577608526749566457456844392655675496443456746"
        "747458655616568356575b13482964a555443592868454663547768437554583146c120",
    ("loop", 10):
        "34a68556a66556651a5466456944545552d6472546856665328684675374546516a5735555695655"
        "406c3467336a6565546743556558a264553577766511985666447457555592545775396543456777"
        "754447655806568366442b73484664b4554445a5565661855556667446554585434b110",
    ("loop", 11):
        "27a6655676935683279466446a17453344a967354585866342596647455954471596735555693546"
        "524c5546424a956544666356660ca154556577608616749566457456254392b55675496442556756"
        "757438655616568356575b13482964a5554435928684546635476584475455834469220",
    ("last", 0):
        "34a68556a66556651a5466456954445555a647254685666442868447547454671695735555696645"
        "406a5466426a7566456643556558a263465388755640965666447459535592545775596343456777"
        "754447655616568366542b73484664a555444295865661965456667446554585444b100",
    ("last", 1):
        "5767766596837695464565566574556557a0854563a7624445d6576451888653a534467556694454"
        "665a6455555657944458754685338575746675463468a5334663a677374495666551486646458963"
        "665579475456586552455a5866445496566615a55655767455565586430g00",
}


def _issue_order(tiles, lag, has_prev, has_next):
    order = [(0, c, b) for c, r in enumerate(tiles) for b in range(NBLK - 1, r - 1, -1)]
    if has_next:
        order += [(1, c, b) for c in range(2) for b in range(NBLK - 1, -1, -1)]
    last = np.cumsum([NBLK - r for r in tiles])
    cut = [lag if has_prev else 0] + [min(int(e) + lag, len(order)) for e in last]
    return [order[cut[t]:cut[t + 1]] for t in range(len(tiles))]


def drain(*jobs):
    for job in jobs:
        for _ in job:
            pass


def lane(c):
    return slice(c * LANES, (c + 1) * LANES)


def _dot(a, b):
    return lax.dot_general(a, b, (((1,), (0,)), ((), ())), preferred_element_type=F32)


def _kernel(x_hbm, w1_hbm, b1_hbm, w2t_hbm, b2_hbm, o_hbm,
            mxu_s, coef_s, bias_s, mean_s, scale_s, lin_s, carry_s,
            x_s, w1_s, b1_s, w2t_s, b2_s, o_s, sem, *norm_s):
    nb, ntok, nch = x_s.shape
    nt = w1_s.shape[1] // LANES
    ngrp = nch // GROUP
    lin = N_VPU
    job_of = np.cumsum(TILES) - 1
    h_s, t_s = norm_s[0::2], norm_s[1::2]
    head = [(c, b) for c in range(2) for b in range(NBLK - 1, -1, -1)][:LAG]
    w2_row = nt * LANES // 2
    act_row = w2_row + nt * 8
    pin_row = act_row + 4 * NCOL * BLK

    first_in = [pltpu.make_async_copy(src, dst, sem.at[i]) for i, (src, dst) in enumerate((
        (x_hbm.at[0:2], x_s.at[0:2]), (b1_hbm, b1_s), (b2_hbm, b2_s), (w1_hbm, w1_s), (w2t_hbm, w2t_s)))]
    rest_in = pltpu.make_async_copy(x_hbm.at[2:nb], x_s.at[2:nb], sem.at[5])
    bulk_out = pltpu.make_async_copy(o_s.at[0:nb - 1], o_hbm.at[0:nb - 1], sem.at[6])
    last_out = pltpu.make_async_copy(o_s.at[nb - 1:nb], o_hbm.at[nb - 1:nb], sem.at[7])

    def w1_tile(c):
        row = lax.broadcasted_iota(jnp.int32, (ntok, LANES), 0)
        b1 = jnp.where(row < len(A_PARTS), b1_s[c:c + 1, :].astype(F32), 0.0)
        w1 = w1_s[:, lane(c)].astype(F32)
        return jnp.concatenate([w1, b1], axis=0).astype(BF16)

    def row_mean(x):
        return jnp.broadcast_to(jnp.sum(x, axis=-1, keepdims=True) * (1.0 / nch), (ntok, LANES))

    def row_scale(x, mean):
        centred = x - jnp.concatenate([mean] * (nch // LANES), axis=1)
        return lax.rsqrt(row_mean(centred * centred) + EPS) * GELU_A

    def moments(b):
        x = x_s[b].astype(F32)
        mean = row_mean(x)
        return mean, row_scale(x, mean)

    def region(name, zero, batches, slot0):
        start = functools.lru_cache(None)(lambda r: pl.multiple_of(zero * 8 + r, 8))
        rows = lambda r, n: pl.ds(start(r), n)
        pins = [0]

        def pin(vs):
            at = []
            for v in vs:
                at.append(pin_row + 8 * pins[0])
                mxu_s[rows(at[-1], 8), :] = v
                pins[0] = (pins[0] + 1) % NPIN
            return at

        def normalise(b, slot, stats=None):
            for i in range(nch // (2 * LANES)):
                if stats is None:
                    bi = b + (zero >> i)
                    at = pl.ds(pl.multiple_of(bi * ntok, ntok), ntok)
                mean, scale = (jnp.concatenate([v, v], axis=1) for v in stats or (mean_s[at, :], scale_s[at, :]))
                cols = slice(2 * LANES * i, 2 * LANES * (i + 1))
                h = ((x_s[b if stats else bi, :, cols].astype(F32) - mean) * scale).astype(BF16).astype(F32)
                h_s[slot][rows(0, ntok), cols] = h
                b11, b21 = h[0:8, :LANES], h[8:16, :LANES]
                b12, b22 = h[0:8, LANES:], h[8:16, LANES:]
                t1 = b12 - b11
                t2 = b22 - t1
                for k, t in enumerate((b11, b21, t2, t1, b22, b22 - b12, b21 - t2)):
                    t_s[slot][rows(8 * k, 8), lane(i)] = t
                for n in range(8 if stats else NORM_PACE):
                    yield
                    if n == 1:
                        pin([t_s[slot][STEPS:, :LANES], h_s[slot][ntok:, :LANES]])

        def bulk_moments():
            per = LANES // ntok
            for out in (mean_s, scale_s):
                for i in range(nb // per):
                    sums = []
                    for b in range(per * i, per * (i + 1)):
                        x = x_s[b].astype(F32)
                        xs = [x[:, j:j + LANES] for j in range(0, nch, LANES)]
                        if out is scale_s:
                            xs = [v - mean_s[ntok * b:ntok * (b + 1), :] for v in xs]
                            xs = [v * v for v in xs]
                        sums.append(functools.reduce(lambda p, v: p + v, xs))
                        pin([sums[-1][0:8], sums[-1][8:16]])
                        for _ in range(STATS_PACE[out is scale_s]):
                            yield
                    m = jnp.sum(jnp.concatenate(sums, axis=0).T, axis=0, keepdims=True) * (1.0 / nch)
                    if out is scale_s:
                        m = lax.rsqrt(m + EPS) * GELU_A
                    out[rows(LANES * i, LANES), :] = jnp.broadcast_to(m, (LANES, LANES)).T
                for _ in range(STATS_PACE[2]):
                    yield

        def build_table(q, w, extra=None):
            col = lambda s: jnp.broadcast_to(w[:, s:s + 1], (BLK, LANES)).astype(F32)
            for s in range(8):
                lo, hi = col(s), col(s + 8)
                a11, a21, a12, a22 = lo[0:8], lo[8:16], hi[0:8], hi[8:16]
                s1 = a21 + a22
                s2 = s1 - a11
                for k, v in enumerate((a11, a12, s2, s1, a12 - s2, a11 - a21, a22)):
                    coef_s[rows(8 * (STEPS * q + 8 * k + s), 8), :] = v
            bias = col(ntok) * GELU_A
            if extra is None:
                bias = jnp.concatenate([bias[0:8], bias[8:16] - bias[0:8]], axis=0)
            else:
                bias = bias + extra
            bias_s[rows(BLK * q, BLK), :] = bias

        def prepare_tile(c):
            wt = w1_tile(c).T
            mxu_s[rows(c * LANES // 2, LANES // 2), 0:2 * ntok] = pltpu.bitcast(wt, F32)
            mxu_s[rows(w2_row + 8 * c, 8), :] = pltpu.bitcast(w2t_s[:, lane(c)], F32)
            if TILES[c]:
                build_table(int(job_of[c]), wt[0:BLK])

        halves = lambda v: [v[:, :LANES], v[:, LANES:]]

        def activate(v, row):
            z = v * (GELU_K + v * v)
            pin(halves(z))
            for _ in range(GELU_DELAY):
                yield
            for p, a in enumerate(halves(v * jnp.tanh(z))):
                mxu_s[rows(row + 2 * BLK * p, 8), :] = a

        def vector_blocks(slot, g, jobs, pending):
            twice = lambda v: jnp.concatenate([v, v], axis=1)
            for q in jobs:
                def product(k, acc, *parked):
                    for s in range(8):
                        if s == RELOAD_AT:
                            back = [jnp.concatenate([mxu_s[r:r + 8, :] for r in at], axis=1) for at in parked]
                        i = STEPS * q + 8 * k + s
                        r = 8 * k + s
                        h = [jnp.broadcast_to(t_s[slot][r:r + 1, lane(c)], (8, LANES)) for c in (2 * g, 2 * g + 1)]
                        term = twice(coef_s[8 * i:8 * i + 8, :]) * jnp.concatenate(h, axis=1)
                        acc = term if acc is None else acc + term
                        if s < 7:
                            yield acc
                    return [acc] + back

                def result(v, half, col):
                    pin(halves(v))
                    if q != lin:
                        pending.append(activate(v, act_row + ((q % 4) * NCOL + col) * BLK + 8 * half))
                    else:
                        for p, u in enumerate(halves(v)):
                            lin_s[rows(8 * half, 8), lane(2 * p + col)] = u

                bias = lambda i: None if q == lin else twice(bias_s[BLK * q + 8 * i:BLK * q + 8 * i + 8, :])
                m1, = yield from product(0, bias(0))
                at_m1 = pin(halves(m1))
                yield
                c11, = yield from product(1, m1)
                result(c11, 0, 0)
                yield
                m6, m1 = yield from product(2, None, at_m1)
                at_u2 = pin(halves(m6 + m1))
                yield
                m5, = yield from product(3, None)
                at_m5 = pin(halves(m5))
                yield
                m53, u2 = yield from product(4, m5, at_u2)
                result(m53 + u2, 0, 1)
                yield
                m7, u2, m5 = yield from product(5, bias(1), at_u2, at_m5)
                u3 = m7 + u2
                result(u3 + m5, 1, 1)
                yield
                c21, = yield from product(6, u3)
                result(c21, 1, 0)
                yield

        act = {} if name == "first" else {cb: carry_s[i] for i, cb in enumerate(head)}
        for ib, b in enumerate(batches):
            slot, side = (slot0 + ib) % NSLOT, []
            for g in range(ngrp):
                warm = name == "first" and g == 0
                end = ib == len(batches) - 1 and g == ngrp - 1
                split = [0] * nt if warm else TILES
                issues = _issue_order(split, LAG, not warm, not (name == "last" and end))
                if warm:
                    n = sum(len(d) + 1 for d in issues)
                    counts = [0] * (n - 16) + [4] * 14 + [0] * 2
                else:
                    counts = [int(c, 36) for c in SLICES[name, ib * ngrp + g]]
                counts = iter(counts)
                pending, done = [], [0]
                work = vector_blocks(slot, g, [lin] + ([] if warm else list(range(lin))), pending)

                def run_slices():
                    for job in side:
                        next(job, None)
                    n = next(counts)
                    done[0] += n
                    for i in range(n):
                        for job in list(pending):
                            if next(job, job) is job:
                                pending.remove(job)
                        partial = next(work, None)
                        if i == n - 1 and partial is not None:
                            pin(halves(partial))

                out_bias = lambda: jnp.concatenate([bias_s[BLK * lin:BLK * (lin + 1), :]] * NCOL, axis=1)
                if warm:
                    first_in[0].wait()
                    drain(normalise(0, slot, moments(0)))
                    for cp in first_in[1:]:
                        cp.wait()
                    rest_in.start()
                    for c in range(PREP_AHEAD):
                        prepare_tile(c)
                    w1a = jnp.concatenate([w1_tile(c) for c in range(nt)], axis=1)
                    w21 = lax.dot_general(w2t_s[...], w1a, (((1,), (1,)), ((), ())), preferred_element_type=F32)
                    acc = jnp.concatenate([t_s[slot][STEPS:, :]] * 2, axis=0)
                else:
                    acc = out_bias()
                for t in range(nt):
                    if name == "loop" and (g, t) == NORM_AT:
                        side.append(normalise(b + 1, (slot + 1) % NSLOT))
                    for nxt in (0, 1):
                        part = [e[1:] for e in issues[t] if e[0] == nxt]
                        if not part:
                            continue
                        lhs = []
                        for c, blk in part:
                            r = (c * NBLK + blk) * 8
                            lhs.append(mxu_s[r:r + 8, 0:KAUG])
                            run_slices()
                        g2 = (g + nxt) % ngrp
                        h = h_s[(slot + (g + nxt) // ngrp) % NSLOT][:, g2 * GROUP:(g2 + 1) * GROUP]
                        v = _dot(pltpu.bitcast(jnp.concatenate(lhs, axis=0), BF16), h)
                        v = v * jnp.tanh(v * (GELU_K + v * v))
                        for i, cb in enumerate(part):
                            a = v[i * BLK:(i + 1) * BLK]
                            if nxt and end:
                                carry_s[head.index(cb)] = a
                            else:
                                act[cb] = a
                    if split[t]:
                        assert GELU_DELAY < done[0] - (job_of[t] + 2) * STEPS <= 3 * STEPS
                        r = act_row + (int(job_of[t]) % 4) * NCOL * BLK
                        act[t, 0] = jnp.concatenate(
                            [mxu_s[r + BLK * j:r + BLK * (j + 1), :] for j in range(NCOL)], axis=1)
                    hidden = jnp.concatenate([act.pop((t, blk)) for blk in range(NBLK)], axis=0)
                    acc = acc + _dot(pltpu.bitcast(mxu_s[w2_row + 8 * t:w2_row + 8 * t + 8, :], BF16), hidden)
                    run_slices()
                    if warm:
                        if t + PREP_AHEAD < nt:
                            prepare_tile(t + PREP_AHEAD)
                        if t == LIN_AT:
                            eye = (lax.broadcasted_iota(jnp.int32, (ntok, ntok), 0)
                                   == lax.broadcasted_iota(jnp.int32, (ntok, ntok), 1))
                            b2 = jnp.sum(jnp.where(eye, b2_s[...].astype(F32), 0.0), axis=1, keepdims=True)
                            build_table(lin, w21, b2 * (2 * GELU_A))
                            side.append(normalise(1, (slot + 1) % NSLOT, moments(1)))
                        if t == STATS_AT:
                            rest_in.wait()
                            side.append(bulk_moments())
                if warm or g == ngrp - 1:
                    drain(*side)
                if warm:
                    acc = acc + out_bias()
                assert done[0] >= STEPS
                acc = acc + lin_s[...]
                o_s[b, :, g * GROUP:(g + 1) * GROUP] = (acc * (0.5 / GELU_A)).astype(o_s.dtype)

    for cp in first_in:
        cp.start()
    row = lax.broadcasted_iota(jnp.int32, (KAUG - ntok, nch), 0)
    ones = jnp.zeros(row.shape, F32)
    for i, a in enumerate(A_PARTS):
        ones = jnp.where(row == i, a, ones)
    for h, t in zip(h_s, t_s):
        h[ntok:, :] = ones
        t[STEPS:, :] = jnp.zeros((8, nch // 2), F32)
    trips = (nb - 2) // UNROLL

    def body(it, carry):
        zero = it >> 20

        @pl.when(it == 0)
        def _():
            region("first", zero, [0], 0)

        region("loop", zero, [1 + it * UNROLL + i for i in range(UNROLL)], 1)

        @pl.when(it == trips - 1)
        def _():
            bulk_out.start()
            region("last", zero, [nb - 1], 1)

        return carry

    lax.fori_loop(0, trips, body, 0)
    last_out.start()
    bulk_out.wait()
    last_out.wait()


@jax.jit
def pallas_standalone__mixer_token_mlp__sampling_kernel(x, w1, b1, w2, b2):
    nb, ntok, nch = x.shape
    nf = w1.shape[1]
    assert ntok == BLK and nch == 2 * GROUP and nf == LANES * len(TILES)
    assert UNROLL % NSLOT == 0 and (nb - 2) % UNROLL == 0
    args = (x, w1, b1.reshape(nf // LANES, LANES), w2.T, b2.reshape(1, ntok))
    hbm = pl.BlockSpec(memory_space=pltpu.HBM)
    vmem = lambda *shape: pltpu.VMEM(shape, F32)
    return pl.pallas_call(
        _kernel,
        in_specs=[hbm] * len(args),
        out_specs=hbm,
        out_shape=jax.ShapeDtypeStruct(x.shape, x.dtype),
        scratch_shapes=[
            vmem(nf // 2 + nf // 16 + 4 * NCOL * BLK + 8 * NPIN, LANES),
            vmem(8 * STEPS * (N_VPU + 1), LANES),
            vmem(BLK * (N_VPU + 1), LANES),
            vmem(nb * ntok, LANES), vmem(nb * ntok, LANES), vmem(ntok, GROUP), vmem(LAG, BLK, GROUP),
        ] + [pltpu.VMEM(a.shape, a.dtype) for a in args] + [
            pltpu.VMEM(x.shape, x.dtype), pltpu.SemaphoreType.DMA((8,)),
        ] + [vmem(KAUG, nch), vmem(STEPS + 8, nch // 2)] * NSLOT,
        compiler_params=pltpu.CompilerParams(vmem_limit_bytes=128 * 2**20),
    )(*args)
```
